```python
import os as _os
_os.environ.setdefault("JAX_PLATFORMS", "cpu")
import jax
import jax.numpy as jnp

def _softmax(x, axis=-1):
    return jax.nn.softmax(x, axis=axis)
def _gelu(x):
    return jax.nn.gelu(x, approximate=True)
def _silu(x):
    return jax.nn.silu(x)
def _sigmoid(x):
    return jax.nn.sigmoid(x)
def _layernorm(x, axis=-1, eps=1e-5):
    m = jnp.mean(x, axis=axis, keepdims=True)
    v = jnp.var(x, axis=axis, keepdims=True)
    return (x - m) / jnp.sqrt(v + eps)
def _scatter_add(tgt, idx, src, axis=0):
    return tgt.at[idx].add(src)
def _segment_sum(src, seg, n):
    return jax.ops.segment_sum(src, seg, n)
class _Rng:
    def __init__(self, key):
        self._k = key
    def _next(self):
        self._k, sub = jax.random.split(self._k)
        return sub
    def normal(self, shape):
        return jax.random.normal(self._next(), shape, dtype=jnp.bfloat16)
    def randint(self, lo, hi, shape):
        return jax.random.randint(self._next(), shape, lo, hi, dtype=jnp.int32)
    def uniform(self, shape, lo=0.0, hi=1.0):
        return jax.random.uniform(self._next(), shape, jnp.bfloat16, lo, hi)
    def permutation(self, n):
        return jax.random.permutation(self._next(), n)


kernel_name = 'parallel_sum__softmax_full_mha__moe_arch_mod__prompt'

def setup_inputs():
    _rng = _Rng(jax.random.key(int.from_bytes(__import__("os").urandom(4), "little")))
    _w = (lambda a: (lambda t: t.astype(jnp.bfloat16) if jnp.issubdtype(t.dtype, jnp.floating) else t)(jnp.asarray(a)))
    def _A_setup():
        B, S, D = 1, 2048, 512
        return {
            "x": _w((lambda *s: _rng.normal(s) * 0.05)(B, S, D)),
            "wqkv": _w((lambda *s: _rng.normal(s) * 0.1)(D, 3 * D)),
            "wo": _w((lambda *s: _rng.normal(s) * 0.05)(D, D)),
        }
    _A_in = _A_setup()

    def _B_setup():
        B, S, D, F, C = 1, 2048, 512, 1792, 1
        return {
            "x": _w((lambda *s: _rng.normal(s) * 0.05)(B, S, D)),
            "w_r": _w((lambda *s: _rng.normal(s) * 1.6)(D)),
            "w_gate": _w((lambda *s: _rng.normal(s) * 0.1)(D, F)),
            "w_up": _w((lambda *s: _rng.normal(s) * 0.1)(D, F)),
            "w_down": _w((lambda *s: _rng.normal(s) * 0.1)(F, D)),
        }
    _B_in = _B_setup()

    return {
        "A_x": _A_in["x"],
        "A_wqkv": _A_in["wqkv"],
        "A_wo": _A_in["wo"],
        "B_x": _B_in["x"],
        "B_w_r": _B_in["w_r"],
        "B_w_gate": _B_in["w_gate"],
        "B_w_up": _B_in["w_up"],
        "B_w_down": _B_in["w_down"],
    }

def reference(A_x, A_wqkv, A_wo, B_x, B_w_r, B_w_gate, B_w_up, B_w_down):
    def _A_ref(x, wqkv, wo):
        B, S, D = x.shape
        H = 32; Dh = D // H
        qkv = (lambda x, *d: x.transpose(*d))((x @ wqkv).reshape(B, S, 3, H, Dh), 2, 0, 3, 1, 4)
        q, k, v = qkv[0], qkv[1], qkv[2]
        scale = Dh ** -0.5
        scores = jnp.einsum("bhqd,bhkd->bhqk", q, k) * scale
        p = _softmax(scores, axis=-1)
        o = jnp.einsum("bhqk,bhkd->bhqd", p, v)
        return (lambda x, *d: x.transpose(*d))(o, 0, 2, 1, 3).reshape(B, S, D) @ wo

    def _B_ref(x, w_r, w_gate, w_up, w_down):
        B, S, D = x.shape
        C = 1
        r = x @ w_r
        idx = jnp.argsort(-r, axis=-1)[:, :C]
        idx_e = jnp.repeat(idx.reshape(B, C, 1), D, axis=2)
        x_sel = jnp.take_along_axis(x, idx_e, axis=1)
        g = _silu(x_sel @ w_gate)
        u = x_sel @ w_up
        y = (g * u) @ w_down
        r_sel = _sigmoid(jnp.take_along_axis(r, idx, axis=1))
        y = y * r_sel.reshape(B, C, 1)
        b_off = (jnp.arange(B) * S).reshape(B, 1)
        flat_idx = (idx + b_off).reshape(B * C)
        zero = (x * 0.0).reshape(B * S, D)
        upd = _scatter_add(zero, flat_idx, y.reshape(B * C, D), axis=0)
        return x + upd.reshape(B, S, D)

    x = A_x
    xn = _layernorm(x, axis=-1)
    return x + _A_ref(xn, A_wqkv, A_wo) + _B_ref(xn, B_w_r, B_w_gate, B_w_up, B_w_down)
```

```python
import jax
import jax.numpy as jnp
from jax import lax
import jax.experimental.pallas as pl
import jax.experimental.pallas.tpu as pltpu

S = 2048
D = 512
H = 32
DH = 16
F = 1792
TQ = 512
KC = 128
LAG = 1
U = 4
ZACC = 1
EXP2 = 1
NQ = S // TQ
NC = S // KC
NB = H // U
EPS = 1e-5
LOG2E = 1.4426950408889634
f32 = jnp.float32
bf16 = jnp.bfloat16


def _kernel(x_ref, wqkv_ref, wr_ref, wo_hbm, wg_hbm, wu_hbm, wd_hbm, o_ref,
            xn_s, k_s, qt_s, vt_s, ot_s, y_s, idx_s, wo_s, wg_s, wu_s, wd_s, sems, *bufs):
    qi = pl.program_id(0)
    sbuf = [bufs[0:U], bufs[U:2 * U]]
    mbuf = [bufs[2 * U:3 * U], bufs[3 * U:4 * U]]

    copies = [pltpu.make_async_copy(src, dst, sems.at[i]) for i, (src, dst) in enumerate(
        [(wg_hbm, wg_s), (wu_hbm, wu_s), (wd_hbm, wd_s), (wo_hbm, wo_s)])]

    def get_w(t):
        q = t // H
        h = t % H
        g = h // 8
        hh = h % 8
        qt = qt_s[q, pl.ds(pl.multiple_of(g * 128, 128), 128), :]
        rows = lax.broadcasted_iota(jnp.int32, (128, TQ), 0) // DH
        w = jnp.where(rows == hh, qt, jnp.zeros_like(qt))
        return g, w

    def produce_only(t, s_ref, m_ref):
        g, w = get_w(t)
        s = jnp.dot(k_s[g], w, preferred_element_type=f32)
        s_ref[...] = s
        m_ref[...] = jnp.max(s, axis=0, keepdims=True)

    def p_chunk(c, s_ref, m8, lsum):
        sl = pl.ds(c * KC, KC)
        z = s_ref[sl, :].reshape(KC // 8, 8, TQ) - m8[None]
        pf = jnp.exp2(z) if EXP2 else jnp.exp(z)
        p = pf.reshape(KC, TQ).astype(bf16)
        cs = None
        for i in reversed(range(KC // 8)):
            cs = pf[i] if cs is None else cs + pf[i]
        lsum = cs if lsum is None else lsum + cs
        return p, lsum

    def pv_chunk(h, c, p, acc):
        sl = pl.ds(c * KC, KC)
        hrow = pl.multiple_of(h * DH, DH)
        vt = vt_s[pl.ds(hrow, DH), sl]
        r = jnp.dot(vt, p, preferred_element_type=f32)
        return r if acc is None else acc + r

    def finalize(h, acc, lsum):
        hrow = pl.multiple_of(h * DH, DH)
        o = acc / jnp.sum(lsum, axis=0, keepdims=True)
        ot_s[pl.ds(hrow, DH), :] = o.astype(bf16)

    def unit(h, sc_ref, m_cur, sn_ref, mn_ref, sp_ref, m_prev, acc_p, lsum_p, produce):
        if produce:
            g, w = get_w(qi * H + h + U)
        hp = jnp.maximum(h - 1, 0)
        mx = None
        acc = jnp.zeros((DH, TQ), f32) if ZACC else None
        lsum = jnp.zeros((8, TQ), f32) if ZACC else None
        for c in range(NC):
            sl = pl.ds(c * KC, KC)
            if c < LAG:
                p, lsum_p = p_chunk(NC - LAG + c, sp_ref, m_prev, lsum_p)
            else:
                p, lsum = p_chunk(c - LAG, sc_ref, m_cur, lsum)
            if produce:
                s = jnp.dot(k_s[g, sl, :], w, preferred_element_type=f32)
                sn_ref[sl, :] = s
                cm = jnp.max(s.reshape(KC // 8, 8, TQ), axis=0)
                mx = cm if mx is None else jnp.maximum(mx, cm)
            if c < LAG:
                acc_p = pv_chunk(hp, NC - LAG + c, p, acc_p)
                if c == LAG - 1:
                    finalize(hp, acc_p, lsum_p)
            else:
                acc = pv_chunk(h, c - LAG, p, acc)
        if produce:
            mn_ref[...] = jnp.max(mx, axis=0, keepdims=True)
        return acc, lsum

    def block(b, par, acc_p, lsum_p, produce=True):
        ms = [jnp.broadcast_to(mbuf[par][u][...], (8, TQ)) for u in range(U)]
        m_prev = jnp.broadcast_to(mbuf[1 - par][U - 1][...], (8, TQ))
        sp_ref = sbuf[1 - par][U - 1]
        for u in range(U):
            h = b * U + u
            acc_p, lsum_p = unit(h, sbuf[par][u], ms[u], sbuf[1 - par][u], mbuf[1 - par][u],
                                 sp_ref, m_prev, acc_p, lsum_p, produce)
            sp_ref = sbuf[par][u]
            m_prev = ms[u]
        return acc_p, lsum_p

    @pl.when(qi == 0)
    def _prologue():
        for cp in copies:
            cp.start()
        x = x_ref[...].astype(f32)
        mean = jnp.mean(x, axis=-1, keepdims=True)
        xc = x - mean
        var = jnp.mean(xc * xc, axis=-1, keepdims=True)
        m_b = mean.astype(bf16).astype(f32)
        v_b = var.astype(bf16).astype(f32)
        d = (x - m_b).astype(bf16).astype(f32)
        den = jnp.sqrt((v_b + EPS).astype(bf16).astype(f32)).astype(bf16).astype(f32)
        xn = (d / den).astype(bf16)
        xn_s[...] = xn
        k = jnp.dot(xn, wqkv_ref[:, D:2 * D], preferred_element_type=f32).astype(bf16)
        for g in range(4):
            k_s[g] = k[:, g * 128:(g + 1) * 128]
        nt = (((0,), (1,)), ((), ()))
        qt = lax.dot_general(wqkv_ref[:, 0:D], xn, nt, preferred_element_type=f32)
        if EXP2:
            qt = (qt * (0.25 * LOG2E)).astype(bf16)
        else:
            qt = (qt * 0.25).astype(bf16)
        for q in range(NQ):
            qt_s[q] = qt[:, q * TQ:(q + 1) * TQ]
        vt = lax.dot_general(wqkv_ref[:, 2 * D:3 * D], xn, nt, preferred_element_type=f32)
        vt_s[...] = vt.astype(bf16)
        for u in range(U):
            produce_only(u, sbuf[0][u], mbuf[0][u])
        sbuf[1][U - 1][pl.ds((NC - LAG) * KC, LAG * KC), :] = jnp.zeros((LAG * KC, TQ), f32)
        mbuf[1][U - 1][...] = jnp.zeros((1, TQ), f32)
        wr8 = jnp.broadcast_to(wr_ref[...], (8, D))
        r = lax.dot_general(wr8, xn, (((1,), (1,)), ((), ())), preferred_element_type=f32)
        r = r.astype(bf16).astype(f32)
        r = jnp.where(r != r, -jnp.inf, r)
        rmax = jnp.max(r, axis=1, keepdims=True)
        lane = lax.broadcasted_iota(jnp.int32, (8, S), 1)
        idx = jnp.min(jnp.where(r == rmax, lane, S), axis=1, keepdims=True)
        onehot = jnp.where(lane == idx, 1.0, 0.0).astype(bf16)
        xsel = jnp.dot(onehot, xn, preferred_element_type=f32).astype(bf16)
        for cp in copies:
            cp.wait()
        a = jnp.dot(xsel, wg_s[...], preferred_element_type=f32).astype(bf16).astype(f32)
        gte = (a * jax.nn.sigmoid(a)).astype(bf16).astype(f32)
        u = jnp.dot(xsel, wu_s[...], preferred_element_type=f32).astype(bf16).astype(f32)
        gu = (gte * u).astype(bf16)
        y = jnp.dot(gu, wd_s[...], preferred_element_type=f32).astype(bf16).astype(f32)
        rs = jax.nn.sigmoid(rmax).astype(bf16).astype(f32)
        y_s[...] = (y * rs).astype(bf16).astype(f32)
        idx_s[...] = jnp.broadcast_to(idx, (8, 128))

    def body(b, carry):
        return lax.cond(
            b % 2 == 0,
            lambda a, l: block(b, 0, a, l),
            lambda a, l: block(b, 1, a, l),
            *carry)

    init = (jnp.zeros((DH, TQ), f32), jnp.ones((8, TQ), f32))
    is_last = qi == NQ - 1
    carry = lax.fori_loop(0, NB - is_last.astype(jnp.int32), body, init)
    acc_p, lsum_p = lax.cond(
        is_last,
        lambda a, l: block(NB - 1, (NB - 1) % 2, a, l, produce=False),
        lambda a, l: (a, l),
        *carry)
    lp = (NB - 1) % 2
    m_prev = jnp.broadcast_to(mbuf[lp][U - 1][...], (8, TQ))
    for c in range(LAG):
        p, lsum_p = p_chunk(NC - LAG + c, sbuf[lp][U - 1], m_prev, lsum_p)
        acc_p = pv_chunk(H - 1, NC - LAG + c, p, acc_p)
    finalize(H - 1, acc_p, lsum_p)

    attn = lax.dot_general(ot_s[...], wo_s[...], (((0,), (0,)), ((), ())),
                           preferred_element_type=f32)
    row0 = pl.multiple_of(qi * TQ, TQ)
    xq = x_ref[pl.ds(row0, TQ), :].astype(f32)
    xnq = xn_s[pl.ds(row0, TQ), :].astype(f32)
    rows = lax.broadcasted_iota(jnp.int32, (TQ, D), 0) + qi * TQ
    upd = jnp.where(rows == idx_s[0:1, 0:1], y_s[0:1, :], 0.0)
    o_ref[...] = ((xq + attn) + (xnq + upd)).astype(o_ref.dtype)


@jax.jit
def pallas_parallel_sum__softmax_full_mha__moe_arch_mod__prompt_kernel(
    A_x, A_wqkv, A_wo, B_x, B_w_r, B_w_gate, B_w_up, B_w_down,
):
    x = A_x.reshape(S, D)
    wr = B_w_r.reshape(1, D)
    full = lambda shape: pl.BlockSpec(shape, lambda i: (0,) * len(shape))
    anyspec = pl.BlockSpec(memory_space=pl.ANY)
    out = pl.pallas_call(
        _kernel,
        grid=(NQ,),
        in_specs=[full((S, D)), full((D, 3 * D)), full((1, D)),
                  anyspec, anyspec, anyspec, anyspec],
        out_specs=pl.BlockSpec((TQ, D), lambda i: (i, 0)),
        out_shape=jax.ShapeDtypeStruct((S, D), bf16),
        scratch_shapes=[
            pltpu.VMEM((S, D), bf16),
            pltpu.VMEM((4, S, 128), bf16),
            pltpu.VMEM((NQ, D, TQ), bf16),
            pltpu.VMEM((D, S), bf16),
            pltpu.VMEM((D, TQ), bf16),
            pltpu.VMEM((8, D), f32),
            pltpu.VMEM((8, 128), jnp.int32),
            pltpu.VMEM((D, D), bf16),
            pltpu.VMEM((D, F), bf16),
            pltpu.VMEM((D, F), bf16),
            pltpu.VMEM((F, D), bf16),
            pltpu.SemaphoreType.DMA((4,)),
        ] + [pltpu.VMEM((S, TQ), f32) for _ in range(2 * U)]
          + [pltpu.VMEM((1, TQ), f32) for _ in range(2 * U)],
        compiler_params=pltpu.CompilerParams(
            dimension_semantics=("arbitrary",),
            vmem_limit_bytes=110 * 1024 * 1024,
        ),
    )(x, A_wqkv, wr, A_wo, B_w_gate, B_w_up, B_w_down)
    return out.reshape(1, S, D)
```

```python
import jax
import jax.numpy as jnp
from jax import lax
import jax.experimental.pallas as pl
import jax.experimental.pallas.tpu as pltpu

S = 2048
D = 512
H = 32
DH = 16
F = 1792
TQ = 512
KC = 128
U = 4
NQ = S // TQ
NC = S // KC
NB = H // U
NGB = NQ * NB
EPS = 1e-5
LOG2E = 1.4426950408889634
f32 = jnp.float32
bf16 = jnp.bfloat16
MT = 2 * D + 16
KPART = 384


def _kernel(x_hbm, wqkv_hbm, wr_ref, wo_hbm, wg_hbm, wu_hbm, wd_hbm, o_hbm,
            x_s, w_s, wt_s, xn_s, k_s, qt_s, vt_s, r_s, ot_s, y_s, idx_s,
            wo_s, wg_s, wu_s, wd_s, o_s, part_s, w0a_s, w0b_s, mpa_s, mpb_s, sems, osems, *bufs):
    sbuf = [bufs[0:U], bufs[U:2 * U]]
    mbuf = [bufs[2 * U:3 * U], bufs[3 * U:4 * U]]
    w0buf = [w0a_s, w0b_s]
    mpbuf = [mpa_s, mpb_s]

    x_cp = [pltpu.make_async_copy(x_hbm.at[pl.ds(i * TQ, TQ), :], x_s.at[pl.ds(i * TQ, TQ), :], sems.at[i])
            for i in range(NQ)]
    w_cp = [pltpu.make_async_copy(wqkv_hbm.at[:, pl.ds(j * D, D)], w_s.at[:, pl.ds(j * D, D)], sems.at[NQ + n])
            for n, j in enumerate([1, 0, 2])]
    late_cp = [pltpu.make_async_copy(src, dst, sems.at[NQ + 3 + i]) for i, (src, dst) in enumerate(
        [(wg_hbm, wg_s), (wu_hbm, wu_s), (wd_hbm, wd_s), (wo_hbm, wo_s)])]

    def out_cp(q):
        row0 = q * TQ if isinstance(q, int) else pl.multiple_of(q * TQ, TQ)
        return pltpu.make_async_copy(o_s.at[pl.ds(row0, TQ), :], o_hbm.at[pl.ds(row0, TQ), :], osems.at[q])

    def get_w(t):
        q = t // H
        h = t % H
        g = h // 8
        hh = h % 8
        qt = qt_s[q, pl.ds(pl.multiple_of(g * 128, 128), 128), :]
        rows = lax.broadcasted_iota(jnp.int32, (128, TQ), 0) // DH
        w = jnp.where(rows == hh, qt, jnp.zeros_like(qt))
        return g, w

    def produce_only(t, s_ref, m_ref, extra=None, kc=256):
        g, w = get_w(t)
        mx = None
        for c in range(S // kc):
            sl = pl.ds(c * kc, kc)
            s = jnp.dot(k_s[g, sl, :], w, preferred_element_type=f32)
            s_ref[sl, :] = s
            cm = jnp.max(s.reshape(kc // 8, 8, TQ), axis=0)
            mx = cm if mx is None else jnp.maximum(mx, cm)
            if extra is not None:
                extra(c)
        m_ref[...] = mx

    def p_chunk(c, s_ref, m8, lsum):
        sl = pl.ds(c * KC, KC)
        pf = jnp.exp2(s_ref[sl, :].reshape(KC // 8, 8, TQ) - m8[None])
        p = pf.reshape(KC, TQ).astype(bf16)
        cs = None
        for i in reversed(range(KC // 8)):
            cs = pf[i] if cs is None else cs + pf[i]
        lsum = cs if lsum is None else lsum + cs
        return p, lsum

    def hrow_of(t):
        return (t % H) * DH if isinstance(t, int) else pl.multiple_of((t % H) * DH, DH)

    def pv_chunk(t, c, p, acc):
        cq, cr = divmod(c * KC, TQ)
        vt = vt_s[cq, pl.ds(hrow_of(t), DH), pl.ds(cr, KC)]
        r = jnp.dot(vt, p, preferred_element_type=f32)
        return r if acc is None else acc + r

    def finalize(t, acc, lsum):
        o = acc / jnp.sum(lsum, axis=0, keepdims=True)
        ot_s[(t // H) % 2, pl.ds(hrow_of(t), DH), :] = o.astype(bf16)

    def unit(t, sc_ref, m_cur, sn_ref, mn_ref, sp_ref, m_prev, acc_p, lsum_p, produce, extra, w0=None):
        if produce:
            if w0 is not None:
                g = ((t + U) % H) // 8
                w = w0[...]
            else:
                g, w = get_w(t + U)
        tp = max(t - 1, 0) if isinstance(t, int) else jnp.maximum(t - 1, 0)
        mx = None
        acc = None
        lsum = None
        for c in range(NC):
            sl = pl.ds(c * KC, KC)
            if c == 0:
                p, lsum_p = p_chunk(NC - 1, sp_ref, m_prev, lsum_p)
            else:
                p, lsum = p_chunk(c - 1, sc_ref, m_cur, lsum)
            if produce:
                s = jnp.dot(k_s[g, sl, :], w, preferred_element_type=f32)
                sn_ref[sl, :] = s
                cm = jnp.max(s.reshape(KC // 8, 8, TQ), axis=0)
                mx = cm if mx is None else jnp.maximum(mx, cm)
            if extra is not None:
                extra(c)
            if c == 0:
                acc_p = pv_chunk(tp, NC - 1, p, acc_p)
                finalize(tp, acc_p, lsum_p)
            else:
                acc = pv_chunk(t, c - 1, p, acc)
        if produce:
            mn_ref[...] = mx
        return acc, lsum

    def block(gb, par, acc_p, lsum_p, produce=True, extras=None):
        ms = [jnp.broadcast_to(jnp.max(mbuf[par][u][...], axis=0, keepdims=True), (8, TQ)) for u in range(U)]
        m_prev = mpbuf[1 - par][...]
        mpbuf[par][...] = ms[U - 1]
        sp_ref = sbuf[1 - par][U - 1]
        for u in range(U):
            t = gb * U + u
            acc_p, lsum_p = unit(t, sbuf[par][u], ms[u], sbuf[1 - par][u], mbuf[1 - par][u],
                                 sp_ref, m_prev, acc_p, lsum_p, produce,
                                 None if extras is None else extras[u],
                                 w0buf[par] if u == 0 else None)
            sp_ref = sbuf[par][u]
            m_prev = ms[u]
            if produce and u == 1:
                tw = jnp.minimum((gb + 2) * U, NQ * H - 1)
                w0buf[1 - par][...] = get_w(tw)[1]
        return acc_p, lsum_p

    tn = (((0,), (0,)), ((), ()))

    def out_rows(q, r0, n, attn):
        base = q * TQ + r0
        if not isinstance(base, int):
            base = pl.multiple_of(base, 128)
        xq = x_s[pl.ds(base, n), :].astype(f32)
        xnq = xn_s[pl.ds(base, n), :].astype(f32)
        rows = lax.broadcasted_iota(jnp.int32, (n, D), 0) + base
        upd = jnp.where(rows == idx_s[0:1, 0:1], y_s[0:1, :], 0.0)
        o_s[pl.ds(base, n), :] = ((xq + attn) + (xnq + upd)).astype(bf16)

    def epilogue(q):
        attn = lax.dot_general(ot_s[q % 2], wo_s[...], tn, preferred_element_type=f32)
        out_rows(q, 0, TQ, attn)
        out_cp(q).start()

    def layernorm(i):
        sl = pl.ds(i * TQ, TQ)
        x = x_s[sl, :].astype(f32)
        mean = jnp.mean(x, axis=-1, keepdims=True)
        xc = x - mean
        var = jnp.mean(xc * xc, axis=-1, keepdims=True)
        m_b = mean.astype(bf16).astype(f32)
        v_b = var.astype(bf16).astype(f32)
        d = (x - m_b).astype(bf16).astype(f32)
        den = jnp.sqrt((v_b + EPS).astype(bf16).astype(f32)).astype(bf16).astype(f32)
        xn_s[sl, :] = (d * (1.0 / den)).astype(bf16)

    def proj_k(i):
        sl = pl.ds(i * TQ, TQ)
        k = jnp.dot(xn_s[sl, :], w_s[:, D:2 * D], preferred_element_type=f32).astype(bf16)
        for g in range(4):
            k_s[g, sl, :] = k[:, g * 128:(g + 1) * 128]

    def proj_t(i):
        sl = pl.ds(i * TQ, TQ)
        t = lax.dot_general(wt_s[...], xn_s[sl, :], (((1,), (1,)), ((), ())),
                            preferred_element_type=f32)
        qt_s[i] = (t[0:D] * (0.25 * LOG2E)).astype(bf16)
        vt_s[i] = t[D:2 * D].astype(bf16)
        r_s[:, sl] = t[2 * D:2 * D + 8]

    x_cp[0].start()
    for cp in w_cp:
        cp.start()
    for i in range(1, NQ):
        x_cp[i].start()
    for cp in late_cp:
        cp.start()
    x_cp[0].wait()
    layernorm(0)
    w_cp[0].wait()
    proj_k(0)
    w_cp[1].wait()
    w_cp[2].wait()
    wt_s[0:D, :] = w_s[:, 0:D].T
    wt_s[D:2 * D, :] = w_s[:, 2 * D:3 * D].T
    wt_s[2 * D:MT, :] = jnp.broadcast_to(wr_ref[...], (16, D))
    for i in range(1, NQ):
        x_cp[i].wait()
        layernorm(i)
        proj_t(i - 1)
        proj_k(i)
    proj_t(NQ - 1)
    sbuf[1][U - 1][pl.ds((NC - 1) * KC, KC), :] = jnp.zeros((KC, TQ), f32)
    mpbuf[1][...] = jnp.zeros((8, TQ), f32)
    w0buf[0][...] = get_w(U)[1]
    for cp in late_cp:
        cp.wait()
    r = r_s[...].astype(bf16).astype(f32)
    r = jnp.where(r != r, -jnp.inf, r)
    rmax = jnp.max(r, axis=1, keepdims=True)
    lane = lax.broadcasted_iota(jnp.int32, (8, S), 1)
    idx = jnp.min(jnp.where(r == rmax, lane, S), axis=1, keepdims=True)
    onehot = jnp.where(lane == idx, 1.0, 0.0).astype(bf16)
    idx_s[...] = jnp.broadcast_to(idx, (8, 128))
    st = {}

    def ex_sel(c):
        part = jnp.dot(onehot[:, c * 256:(c + 1) * 256], xn_s[pl.ds(c * 256, 256), :],
                       preferred_element_type=f32)
        st['xsel'] = part if c == 0 else st['xsel'] + part

    nsplit = [0, 512, 1024, 1536, 1792]

    def ex_gu(c):
        if c == 0:
            st['xs'] = st['xsel'].astype(bf16)
        wref = wg_s if c < 4 else wu_s
        j = c % 4
        st[c] = jnp.dot(st['xs'], wref[:, nsplit[j]:nsplit[j + 1]],
                        preferred_element_type=f32).astype(bf16).astype(f32)

    def ex_down(c):
        if c == 0:
            a = jnp.concatenate([st[j] for j in range(4)], axis=1)
            u_ = jnp.concatenate([st[4 + j] for j in range(4)], axis=1)
            gte = (a * jax.nn.sigmoid(a)).astype(bf16).astype(f32)
            st['gu'] = (gte * u_).astype(bf16)
        if c < 7:
            part = jnp.dot(st['gu'][:, c * 256:(c + 1) * 256], wd_s[pl.ds(c * 256, 256), :],
                           preferred_element_type=f32)
            st['y'] = part if c == 0 else st['y'] + part

    extras = [None, ex_sel, ex_gu, ex_down]
    for u in range(U):
        produce_only(u, sbuf[0][u], mbuf[0][u], extras[u])
    y = st['y'].astype(bf16).astype(f32)
    rs = jax.nn.sigmoid(rmax).astype(bf16).astype(f32)
    y_s[...] = (y * rs).astype(bf16).astype(f32)

    def body(gb, carry):
        carry = lax.cond(
            gb % 2 == 0,
            lambda a, l: block(gb, 0, a, l),
            lambda a, l: block(gb, 1, a, l),
            *carry)

        @pl.when(jnp.logical_and(gb % NB == 0, jnp.logical_and(gb > 0, gb < (NQ - 1) * NB)))
        def _():
            epilogue(gb // NB - 1)

        return carry

    init = (jnp.zeros((DH, TQ), f32), jnp.ones((8, TQ), f32))
    acc_p, lsum_p = lax.fori_loop(0, NGB - 1, body, init)

    qa = NQ - 2
    qb = NQ - 1

    RP = 64
    NKA = D // 128
    NKB = KPART // 128
    pieces = [(qa, j, kt) for j in range(TQ // RP) for kt in range(NKA)]
    pieces += [(qb, j, kt) for j in range(TQ // RP) for kt in range(NKB)]
    nslot = U * NC
    pacc = {}

    def mk_ex(u):
        def ex(c):
            s = u * NC + c
            lo = (s * len(pieces)) // nslot
            hi = ((s + 1) * len(pieces)) // nslot
            for (q, j, kt) in pieces[lo:hi]:
                r = lax.dot_general(ot_s[q % 2, pl.ds(kt * 128, 128), pl.ds(j * RP, RP)],
                                    wo_s[pl.ds(kt * 128, 128), :], tn, preferred_element_type=f32)
                pacc[0] = r if kt == 0 else pacc[0] + r
                if q == qa and kt == NKA - 1:
                    out_rows(qa, j * RP, RP, pacc[0])
                if q == qb and kt == NKB - 1:
                    part_s[pl.ds(j * RP, RP), :] = pacc[0]
        return ex

    lb = NGB - 1
    lp = lb % 2
    acc_p, lsum_p = block(lb, lp, acc_p, lsum_p, produce=False,
                          extras=[mk_ex(u) for u in range(U)])
    out_cp(qa).start()
    m_prev = mpbuf[lp][...]
    p, lsum_p = p_chunk(NC - 1, sbuf[lp][U - 1], m_prev, lsum_p)
    acc_p = pv_chunk(NQ * H - 1, NC - 1, p, acc_p)
    finalize(NQ * H - 1, acc_p, lsum_p)
    attn = part_s[...] + lax.dot_general(ot_s[qb % 2, pl.ds(KPART, D - KPART), :],
                                         wo_s[pl.ds(KPART, D - KPART), :], tn,
                                         preferred_element_type=f32)
    out_rows(qb, 0, TQ, attn)
    out_cp(qb).start()
    for q in range(NQ):
        out_cp(q).wait()


@jax.jit
def pallas_parallel_sum__softmax_full_mha__moe_arch_mod__prompt_kernel(
    A_x, A_wqkv, A_wo, B_x, B_w_r, B_w_gate, B_w_up, B_w_down,
):
    x = A_x.reshape(S, D)
    wr = B_w_r.reshape(1, D)
    anyspec = pl.BlockSpec(memory_space=pl.ANY)
    out = pl.pallas_call(
        _kernel,
        in_specs=[anyspec, anyspec, pl.BlockSpec(memory_space=pltpu.VMEM),
                  anyspec, anyspec, anyspec, anyspec],
        out_specs=anyspec,
        out_shape=jax.ShapeDtypeStruct((S, D), bf16),
        scratch_shapes=[
            pltpu.VMEM((S, D), bf16),
            pltpu.VMEM((D, 3 * D), bf16),
            pltpu.VMEM((MT, D), bf16),
            pltpu.VMEM((S, D), bf16),
            pltpu.VMEM((4, S, 128), bf16),
            pltpu.VMEM((NQ, D, TQ), bf16),
            pltpu.VMEM((NQ, D, TQ), bf16),
            pltpu.VMEM((8, S), f32),
            pltpu.VMEM((2, D, TQ), bf16),
            pltpu.VMEM((8, D), f32),
            pltpu.VMEM((8, 128), jnp.int32),
            pltpu.VMEM((D, D), bf16),
            pltpu.VMEM((D, F), bf16),
            pltpu.VMEM((D, F), bf16),
            pltpu.VMEM((F, D), bf16),
            pltpu.VMEM((S, D), bf16),
            pltpu.VMEM((TQ, D), f32),
            pltpu.VMEM((128, TQ), bf16),
            pltpu.VMEM((128, TQ), bf16),
            pltpu.VMEM((8, TQ), f32),
            pltpu.VMEM((8, TQ), f32),
            pltpu.SemaphoreType.DMA((NQ + 7,)),
            pltpu.SemaphoreType.DMA((NQ,)),
        ] + [pltpu.VMEM((S, TQ), f32) for _ in range(2 * U)]
          + [pltpu.VMEM((8, TQ), f32) for _ in range(2 * U)],
        compiler_params=pltpu.CompilerParams(
            vmem_limit_bytes=110 * 1024 * 1024,
        ),
    )(x, A_wqkv, wr, A_wo, B_w_gate, B_w_up, B_w_down)
    return out.reshape(1, S, D)
```

```python
import jax
import jax.numpy as jnp
from jax import lax
import jax.experimental.pallas as pl
import jax.experimental.pallas.tpu as pltpu

S = 2048
D = 512
H = 32
DH = 16
F = 1792
TQ = 512
KC = 128
U = 4
NQ = S // TQ
NC = S // KC
NB = H // U
NGB = NQ * NB
EPS = 1e-5
LOG2E = 1.4426950408889634
f32 = jnp.float32
bf16 = jnp.bfloat16
MT = 2 * D + 16
NDEF = 2
KPART = ((H - U - 1) * DH // 128) * 128


def _kernel(x_hbm, wqkv_hbm, wr_hbm, wo_hbm, wg_hbm, wu_hbm, wd_hbm, o_hbm,
            x_s, wq_s, wk_s, wv_s, wt_s, xn_s, k_s, qt_s, vt_s, r_s, ot_s, y_s, idx_s,
            wo_s, wg_s, wu_s, wd_s, o_s, part_s, wr_ref, w0a_s, w0b_s, mpa_s, mpb_s, sems, osems, *bufs):
    sbuf = [bufs[0:U], bufs[U:2 * U]]
    mbuf = [bufs[2 * U:3 * U], bufs[3 * U:4 * U]]
    w0buf = [w0a_s, w0b_s]
    mpbuf = [mpa_s, mpb_s]

    x_cp = [pltpu.make_async_copy(x_hbm.at[pl.ds(i * TQ, TQ), :], x_s.at[pl.ds(i * TQ, TQ), :], sems.at[i])
            for i in range(NQ)]
    w_cp = [pltpu.make_async_copy(wqkv_hbm.at[:, pl.ds(j * D, D)], dst, sems.at[NQ + n])
            for n, (j, dst) in enumerate([(1, wk_s), (0, wq_s), (2, wv_s)])]
    wr_cp = pltpu.make_async_copy(wr_hbm, wr_ref, sems.at[NQ + 7])
    late_cp = [pltpu.make_async_copy(src, dst, sems.at[NQ + 3 + i]) for i, (src, dst) in enumerate(
        [(wg_hbm, wg_s), (wu_hbm, wu_s), (wd_hbm, wd_s), (wo_hbm, wo_s)])]

    def out_cp(q):
        row0 = q * TQ if isinstance(q, int) else pl.multiple_of(q * TQ, TQ)
        return pltpu.make_async_copy(o_s.at[pl.ds(row0, TQ), :], o_hbm.at[pl.ds(row0, TQ), :], osems.at[q])

    def get_w(t):
        q = t // H
        h = t % H
        g = h // 8
        hh = h % 8
        qt = qt_s[q, pl.ds(pl.multiple_of(g * 128, 128), 128), :]
        rows = lax.broadcasted_iota(jnp.int32, (128, TQ), 0) // DH
        w = jnp.where(rows == hh, qt, jnp.zeros_like(qt))
        return g, w

    def produce_only(t, s_ref, m_ref, extra=None, kc=256):
        g, w = get_w(t)
        mx = None
        for c in range(S // kc):
            sl = pl.ds(c * kc, kc)
            s = jnp.dot(k_s[g, sl, :], w, preferred_element_type=f32)
            s_ref[sl, :] = s
            cm = jnp.max(s.reshape(kc // 8, 8, TQ), axis=0)
            mx = cm if mx is None else jnp.maximum(mx, cm)
            if extra is not None:
                extra(c)
        m_ref[...] = mx

    def p_chunk(c, s_ref, m8, lsum):
        sl = pl.ds(c * KC, KC)
        pf = jnp.exp2(s_ref[sl, :].reshape(KC // 8, 8, TQ) - m8[None])
        p = pf.reshape(KC, TQ).astype(bf16)
        cs = None
        for i in reversed(range(KC // 8)):
            cs = pf[i] if cs is None else cs + pf[i]
        lsum = cs if lsum is None else lsum + cs
        return p, lsum

    def hrow_of(t):
        return (t % H) * DH if isinstance(t, int) else pl.multiple_of((t % H) * DH, DH)

    def pv_chunk(t, c, p, acc):
        cq, cr = divmod(c * KC, TQ)
        vt = vt_s[cq, pl.ds(hrow_of(t), DH), pl.ds(cr, KC)]
        r = jnp.dot(vt, p, preferred_element_type=f32)
        return r if acc is None else acc + r

    def finalize(t, acc, lsum):
        o = acc / jnp.sum(lsum, axis=0, keepdims=True)
        ot_s[t // H, pl.ds(hrow_of(t), DH), :] = o.astype(bf16)

    def unit(t, sc_ref, m_cur, sn_ref, mn_ref, sp_ref, m_prev, acc_p, lsum_p, produce, extra, w0=None):
        if produce:
            if w0 is not None:
                g = ((t + U) % H) // 8
                w = w0[...]
            else:
                g, w = get_w(t + U)
        tp = max(t - 1, 0) if isinstance(t, int) else jnp.maximum(t - 1, 0)
        mx = None
        acc = None
        lsum = None
        for c in range(NC):
            sl = pl.ds(c * KC, KC)
            if c == 0:
                p, lsum_p = p_chunk(NC - 1, sp_ref, m_prev, lsum_p)
            else:
                p, lsum = p_chunk(c - 1, sc_ref, m_cur, lsum)
            if produce:
                s = jnp.dot(k_s[g, sl, :], w, preferred_element_type=f32)
                sn_ref[sl, :] = s
                cm = jnp.max(s.reshape(KC // 8, 8, TQ), axis=0)
                mx = cm if mx is None else jnp.maximum(mx, cm)
            if extra is not None:
                extra(c)
            if c == 0:
                acc_p = pv_chunk(tp, NC - 1, p, acc_p)
                finalize(tp, acc_p, lsum_p)
            else:
                acc = pv_chunk(t, c - 1, p, acc)
        if produce:
            mn_ref[...] = mx
        return acc, lsum

    def block(gb, par, acc_p, lsum_p, produce=True, extras=None):
        ms = [jnp.broadcast_to(jnp.max(mbuf[par][u][...], axis=0, keepdims=True), (8, TQ)) for u in range(U)]
        m_prev = mpbuf[1 - par][...]
        mpbuf[par][...] = ms[U - 1]
        sp_ref = sbuf[1 - par][U - 1]
        for u in range(U):
            t = gb * U + u
            acc_p, lsum_p = unit(t, sbuf[par][u], ms[u], sbuf[1 - par][u], mbuf[1 - par][u],
                                 sp_ref, m_prev, acc_p, lsum_p, produce,
                                 None if extras is None else extras[u],
                                 w0buf[par] if u == 0 else None)
            sp_ref = sbuf[par][u]
            m_prev = ms[u]
            if produce and u == 1:
                tw = jnp.minimum((gb + 2) * U, NQ * H - 1)
                w0buf[1 - par][...] = get_w(tw)[1]
        return acc_p, lsum_p

    tn = (((0,), (0,)), ((), ()))

    def out_rows(q, r0, n, attn):
        base = q * TQ + r0
        if not isinstance(base, int):
            base = pl.multiple_of(base, 128)
        xq = x_s[pl.ds(base, n), :].astype(f32)
        xnq = xn_s[pl.ds(base, n), :].astype(f32)
        rows = lax.broadcasted_iota(jnp.int32, (n, D), 0) + base
        upd = jnp.where(rows == idx_s[0:1, 0:1], y_s[0:1, :], 0.0)
        o_s[pl.ds(base, n), :] = ((xq + attn) + (xnq + upd)).astype(bf16)

    def epilogue(q):
        attn = lax.dot_general(ot_s[q], wo_s[...], tn, preferred_element_type=f32)
        out_rows(q, 0, TQ, attn)
        out_cp(q).start()

    def layernorm(i):
        sl = pl.ds(i * TQ, TQ)
        x = x_s[sl, :].astype(f32)
        mean = jnp.mean(x, axis=-1, keepdims=True)
        xc = x - mean
        var = jnp.mean(xc * xc, axis=-1, keepdims=True)
        m_b = mean.astype(bf16).astype(f32)
        v_b = var.astype(bf16).astype(f32)
        d = (x - m_b).astype(bf16).astype(f32)
        den = jnp.sqrt((v_b + EPS).astype(bf16).astype(f32)).astype(bf16).astype(f32)
        xn_s[sl, :] = (d * (1.0 / den)).astype(bf16)

    def proj_k(i):
        sl = pl.ds(i * TQ, TQ)
        k = jnp.dot(xn_s[sl, :], wk_s[...], preferred_element_type=f32).astype(bf16)
        for g in range(4):
            k_s[g, sl, :] = k[:, g * 128:(g + 1) * 128]

    def proj_t(i):
        sl = pl.ds(i * TQ, TQ)
        t = lax.dot_general(wt_s[...], xn_s[sl, :], (((1,), (1,)), ((), ())),
                            preferred_element_type=f32)
        qt_s[i] = (t[0:D] * (0.25 * LOG2E)).astype(bf16)
        vt_s[i] = t[D:2 * D].astype(bf16)
        r_s[:, sl] = t[2 * D:2 * D + 8]

    x_cp[0].start()
    for cp in w_cp:
        cp.start()
    wr_cp.start()
    for i in range(1, NQ):
        x_cp[i].start()
    for cp in late_cp:
        cp.start()
    x_cp[0].wait()
    layernorm(0)
    w_cp[0].wait()
    proj_k(0)
    w_cp[1].wait()
    w_cp[2].wait()
    wr_cp.wait()
    wt_s[0:D, :] = wq_s[...].T
    wt_s[D:2 * D, :] = wv_s[...].T
    wt_s[2 * D:MT, :] = jnp.broadcast_to(wr_ref[...].astype(f32).reshape(1, D), (16, D)).astype(bf16)
    for i in range(1, NQ):
        x_cp[i].wait()
        layernorm(i)
        proj_t(i - 1)
        proj_k(i)
    proj_t(NQ - 1)
    sbuf[1][U - 1][pl.ds((NC - 1) * KC, KC), :] = jnp.zeros((KC, TQ), f32)
    mpbuf[1][...] = jnp.zeros((8, TQ), f32)
    w0buf[0][...] = get_w(U)[1]
    for cp in late_cp:
        cp.wait()
    r = r_s[...].astype(bf16).astype(f32)
    r = jnp.where(r != r, -jnp.inf, r)
    rmax = jnp.max(r, axis=1, keepdims=True)
    lane = lax.broadcasted_iota(jnp.int32, (8, S), 1)
    idx = jnp.min(jnp.where(r == rmax, lane, S), axis=1, keepdims=True)
    onehot = jnp.where(lane == idx, 1.0, 0.0).astype(bf16)
    idx_s[...] = jnp.broadcast_to(idx, (8, 128))
    st = {}

    def ex_sel(c):
        part = jnp.dot(onehot[:, c * 256:(c + 1) * 256], xn_s[pl.ds(c * 256, 256), :],
                       preferred_element_type=f32)
        st['xsel'] = part if c == 0 else st['xsel'] + part

    nsplit = [0, 512, 1024, 1536, 1792]

    def ex_gu(c):
        if c == 0:
            st['xs'] = st['xsel'].astype(bf16)
        wref = wg_s if c < 4 else wu_s
        j = c % 4
        st[c] = jnp.dot(st['xs'], wref[:, nsplit[j]:nsplit[j + 1]],
                        preferred_element_type=f32).astype(bf16).astype(f32)

    def ex_down(c):
        if c == 0:
            a = jnp.concatenate([st[j] for j in range(4)], axis=1)
            u_ = jnp.concatenate([st[4 + j] for j in range(4)], axis=1)
            gte = (a * jax.nn.sigmoid(a)).astype(bf16).astype(f32)
            st['gu'] = (gte * u_).astype(bf16)
        if c < 7:
            part = jnp.dot(st['gu'][:, c * 256:(c + 1) * 256], wd_s[pl.ds(c * 256, 256), :],
                           preferred_element_type=f32)
            st['y'] = part if c == 0 else st['y'] + part

    extras = [None] * (U - 3) + [ex_sel, ex_gu, ex_down]
    for u in range(U):
        produce_only(u, sbuf[0][u], mbuf[0][u], extras[u])
    y = st['y'].astype(bf16).astype(f32)
    rs = jax.nn.sigmoid(rmax).astype(bf16).astype(f32)
    y_s[...] = (y * rs).astype(bf16).astype(f32)

    def body(gb, carry):
        carry = lax.cond(
            gb % 2 == 0,
            lambda a, l: block(gb, 0, a, l),
            lambda a, l: block(gb, 1, a, l),
            *carry)

        @pl.when(jnp.logical_and(gb % NB == 0, jnp.logical_and(gb > 0, gb < (NQ - NDEF) * NB)))
        def _():
            epilogue(gb // NB - 1)

        return carry

    init = (jnp.zeros((DH, TQ), f32), jnp.ones((8, TQ), f32))
    acc_p, lsum_p = lax.fori_loop(0, NGB - 1, body, init)

    qas = list(range(NQ - 1 - NDEF, NQ - 1))
    qb = NQ - 1

    RP = 64
    NKA = D // 128
    NKB = KPART // 128
    pieces = [(qa, j, kt) for qa in qas for j in range(TQ // RP) for kt in range(NKA)]
    pieces += [(qb, j, kt) for j in range(TQ // RP) for kt in range(NKB)]
    nslot = U * NC
    pacc = {}

    def mk_ex(u):
        def ex(c):
            s = u * NC + c
            lo = (s * len(pieces)) // nslot
            hi = ((s + 1) * len(pieces)) // nslot
            for (q, j, kt) in pieces[lo:hi]:
                r = lax.dot_general(ot_s[q, pl.ds(kt * 128, 128), pl.ds(j * RP, RP)],
                                    wo_s[pl.ds(kt * 128, 128), :], tn, preferred_element_type=f32)
                pacc[0] = r if kt == 0 else pacc[0] + r
                if q != qb and kt == NKA - 1:
                    out_rows(q, j * RP, RP, pacc[0])
                    if j == TQ // RP - 1:
                        out_cp(q).start()
                if q == qb and kt == NKB - 1:
                    part_s[pl.ds(j * RP, RP), :] = pacc[0]
        return ex

    lb = NGB - 1
    lp = lb % 2
    acc_p, lsum_p = block(lb, lp, acc_p, lsum_p, produce=False,
                          extras=[mk_ex(u) for u in range(U)])
    m_prev = mpbuf[lp][...]
    p, lsum_p = p_chunk(NC - 1, sbuf[lp][U - 1], m_prev, lsum_p)
    acc_p = pv_chunk(NQ * H - 1, NC - 1, p, acc_p)
    finalize(NQ * H - 1, acc_p, lsum_p)
    attn = part_s[...] + lax.dot_general(ot_s[qb, pl.ds(KPART, D - KPART), :],
                                         wo_s[pl.ds(KPART, D - KPART), :], tn,
                                         preferred_element_type=f32)
    out_rows(qb, 0, TQ, attn)
    out_cp(qb).start()
    for q in range(NQ):
        out_cp(q).wait()


@jax.jit
def pallas_parallel_sum__softmax_full_mha__moe_arch_mod__prompt_kernel(
    A_x, A_wqkv, A_wo, B_x, B_w_r, B_w_gate, B_w_up, B_w_down,
):
    x = A_x.reshape(S, D)
    wr = B_w_r
    anyspec = pl.BlockSpec(memory_space=pl.ANY)
    out = pl.pallas_call(
        _kernel,
        in_specs=[anyspec, anyspec, anyspec,
                  anyspec, anyspec, anyspec, anyspec],
        out_specs=anyspec,
        out_shape=jax.ShapeDtypeStruct((S, D), bf16),
        scratch_shapes=[
            pltpu.VMEM((S, D), bf16),
            pltpu.VMEM((D, D), bf16),
            pltpu.VMEM((D, D), bf16),
            pltpu.VMEM((D, D), bf16),
            pltpu.VMEM((MT, D), bf16),
            pltpu.VMEM((S, D), bf16),
            pltpu.VMEM((4, S, 128), bf16),
            pltpu.VMEM((NQ, D, TQ), bf16),
            pltpu.VMEM((NQ, D, TQ), bf16),
            pltpu.VMEM((8, S), f32),
            pltpu.VMEM((NQ, D, TQ), bf16),
            pltpu.VMEM((8, D), f32),
            pltpu.VMEM((8, 128), jnp.int32),
            pltpu.VMEM((D, D), bf16),
            pltpu.VMEM((D, F), bf16),
            pltpu.VMEM((D, F), bf16),
            pltpu.VMEM((F, D), bf16),
            pltpu.VMEM((S, D), bf16),
            pltpu.VMEM((TQ, D), f32),
            pltpu.VMEM((D,), bf16),
            pltpu.VMEM((128, TQ), bf16),
            pltpu.VMEM((128, TQ), bf16),
            pltpu.VMEM((8, TQ), f32),
            pltpu.VMEM((8, TQ), f32),
            pltpu.SemaphoreType.DMA((NQ + 8,)),
            pltpu.SemaphoreType.DMA((NQ,)),
        ] + [pltpu.VMEM((S, TQ), f32) for _ in range(2 * U)]
          + [pltpu.VMEM((8, TQ), f32) for _ in range(2 * U)],
        compiler_params=pltpu.CompilerParams(
            vmem_limit_bytes=110 * 1024 * 1024,
        ),
    )(x, A_wqkv, wr, A_wo, B_w_gate, B_w_up, B_w_down)
    return out.reshape(1, S, D)
```

```python
import jax
import jax.numpy as jnp
from jax import lax
import jax.experimental.pallas as pl
import jax.experimental.pallas.tpu as pltpu

S = 2048
D = 512
H = 32
DH = 16
F = 1792
TQ = 512
KC = 128
U = 4
NQ = S // TQ
NC = S // KC
NB = H // U
NGB = NQ * NB
EPS = 1e-5
LOG2E = 1.4426950408889634
f32 = jnp.float32
bf16 = jnp.bfloat16
MT = 2 * D + 16
NDEF = 2
KPART = ((H - U - 1) * DH // 128) * 128


def _kernel(x_hbm, wqkv_hbm, wr_hbm, wo_hbm, wg_hbm, wu_hbm, wd_hbm, o_hbm,
            x_s, wq_s, wk_s, wv_s, wt_s, xn_s, k_s, qt_s, vt_s, r_s, ot_s, y_s, idx_s,
            wo_s, wg_s, wu_s, wd_s, o_s, part_s, wr_ref, w0a_s, w0b_s, mpa_s, mpb_s, zero_s, sems, osems, *bufs):
    sbuf = [bufs[0:U], bufs[U:2 * U]]
    mbuf = [bufs[2 * U:3 * U], bufs[3 * U:4 * U]]
    w0buf = [w0a_s, w0b_s]
    mpbuf = [mpa_s, mpb_s]

    x_cp = [pltpu.make_async_copy(x_hbm.at[pl.ds(i * TQ, TQ), :], x_s.at[pl.ds(i * TQ, TQ), :], sems.at[i])
            for i in range(NQ)]
    w_cp = [pltpu.make_async_copy(wqkv_hbm.at[:, pl.ds(j * D, D)], dst, sems.at[NQ + n])
            for n, (j, dst) in enumerate([(1, wk_s), (0, wq_s), (2, wv_s)])]
    wr_cp = pltpu.make_async_copy(wr_hbm, wr_ref, sems.at[NQ + 7])
    late_cp = [pltpu.make_async_copy(src, dst, sems.at[NQ + 3 + i]) for i, (src, dst) in enumerate(
        [(wg_hbm, wg_s), (wu_hbm, wu_s), (wd_hbm, wd_s), (wo_hbm, wo_s)])]

    def out_cp(q):
        row0 = q * TQ if isinstance(q, int) else pl.multiple_of(q * TQ, TQ)
        return pltpu.make_async_copy(o_s.at[pl.ds(row0, TQ), :], o_hbm.at[pl.ds(row0, TQ), :], osems.at[q])

    def get_w(t):
        q = t // H
        h = t % H
        g = h // 8
        hh = h % 8
        qt = qt_s[q, pl.ds(pl.multiple_of(g * 128, 128), 128), :]
        rows = lax.broadcasted_iota(jnp.int32, (128, TQ), 0) // DH
        w = jnp.where(rows == hh, qt, jnp.zeros_like(qt))
        return g, w

    def produce_only(t, s_ref, m_ref, extra=None, kc=256):
        g, w = get_w(t)
        mx = None
        for c in range(S // kc):
            sl = pl.ds(c * kc, kc)
            s = jnp.dot(k_s[g, sl, :], w, preferred_element_type=f32)
            s_ref[sl, :] = s
            cm = jnp.max(s.reshape(kc // 8, 8, TQ), axis=0)
            mx = cm if mx is None else jnp.maximum(mx, cm)
            if extra is not None:
                extra(c)
        m_ref[...] = mx

    def p_chunk(c, s_ref, m8, lsum):
        sl = pl.ds(c * KC, KC)
        pf = jnp.exp2(s_ref[sl, :].reshape(KC // 8, 8, TQ) - m8[None])
        p = pf.reshape(KC, TQ).astype(bf16)
        cs = None
        for i in reversed(range(KC // 8)):
            cs = pf[i] if cs is None else cs + pf[i]
        lsum = cs if lsum is None else lsum + cs
        return p, lsum

    def hrow_of(t):
        return (t % H) * DH if isinstance(t, int) else pl.multiple_of((t % H) * DH, DH)

    def pv_chunk(t, c, p, acc):
        cq, cr = divmod(c * KC, TQ)
        vt = vt_s[cq, pl.ds(hrow_of(t), DH), pl.ds(cr, KC)]
        r = jnp.dot(vt, p, preferred_element_type=f32)
        return r if acc is None else acc + r

    def finalize(t, acc, lsum):
        o = acc / jnp.sum(lsum, axis=0, keepdims=True)
        ot_s[t // H, pl.ds(hrow_of(t), DH), :] = o.astype(bf16)

    def unit(t, sc_ref, m_cur, sn_ref, mn_ref, sp_ref, m_prev, acc_p, lsum_p, produce, extra, w0=None):
        if produce:
            if w0 is not None:
                g = ((t + U) % H) // 8
                w = w0[...]
            else:
                g, w = get_w(t + U)
        tp = max(t - 1, 0) if isinstance(t, int) else jnp.maximum(t - 1, 0)
        mx = None
        acc = zero_s[...]
        lsum = None
        for c in range(NC):
            sl = pl.ds(c * KC, KC)
            if c == 0:
                p, lsum_p = p_chunk(NC - 1, sp_ref, m_prev, lsum_p)
            else:
                p, lsum = p_chunk(c - 1, sc_ref, m_cur, lsum)
            if produce:
                s = jnp.dot(k_s[g, sl, :], w, preferred_element_type=f32)
                sn_ref[sl, :] = s
                cm = jnp.max(s.reshape(KC // 8, 8, TQ), axis=0)
                mx = cm if mx is None else jnp.maximum(mx, cm)
            if extra is not None:
                extra(c)
            if c == 0:
                acc_p = pv_chunk(tp, NC - 1, p, acc_p)
                finalize(tp, acc_p, lsum_p)
            else:
                acc = pv_chunk(t, c - 1, p, acc)
        if produce:
            mn_ref[...] = mx
        return acc, lsum

    def block(gb, par, acc_p, lsum_p, produce=True, extras=None):
        ms = [jnp.broadcast_to(jnp.max(mbuf[par][u][...], axis=0, keepdims=True), (8, TQ)) for u in range(U)]
        m_prev = mpbuf[1 - par][...]
        mpbuf[par][...] = ms[U - 1]
        sp_ref = sbuf[1 - par][U - 1]
        for u in range(U):
            t = gb * U + u
            acc_p, lsum_p = unit(t, sbuf[par][u], ms[u], sbuf[1 - par][u], mbuf[1 - par][u],
                                 sp_ref, m_prev, acc_p, lsum_p, produce,
                                 None if extras is None else extras[u],
                                 w0buf[par] if u == 0 else None)
            sp_ref = sbuf[par][u]
            m_prev = ms[u]
            if produce and u == 1:
                tw = jnp.minimum((gb + 2) * U, NQ * H - 1)
                w0buf[1 - par][...] = get_w(tw)[1]
        return acc_p, lsum_p

    tn = (((0,), (0,)), ((), ()))

    def out_rows(q, r0, n, attn):
        base = q * TQ + r0
        if not isinstance(base, int):
            base = pl.multiple_of(base, 128)
        xq = x_s[pl.ds(base, n), :].astype(f32)
        xnq = xn_s[pl.ds(base, n), :].astype(f32)
        rows = lax.broadcasted_iota(jnp.int32, (n, D), 0) + base
        upd = jnp.where(rows == idx_s[0:1, 0:1], y_s[0:1, :], 0.0)
        o_s[pl.ds(base, n), :] = ((xq + attn) + (xnq + upd)).astype(bf16)

    def epilogue(q):
        attn = lax.dot_general(ot_s[q], wo_s[...], tn, preferred_element_type=f32)
        out_rows(q, 0, TQ, attn)
        out_cp(q).start()

    def layernorm(i):
        sl = pl.ds(i * TQ, TQ)
        x = x_s[sl, :].astype(f32)
        mean = jnp.mean(x, axis=-1, keepdims=True)
        xc = x - mean
        var = jnp.mean(xc * xc, axis=-1, keepdims=True)
        m_b = mean.astype(bf16).astype(f32)
        v_b = var.astype(bf16).astype(f32)
        d = (x - m_b).astype(bf16).astype(f32)
        den = jnp.sqrt((v_b + EPS).astype(bf16).astype(f32)).astype(bf16).astype(f32)
        xn_s[sl, :] = (d * (1.0 / den)).astype(bf16)

    def proj_k(i):
        sl = pl.ds(i * TQ, TQ)
        k = jnp.dot(xn_s[sl, :], wk_s[...], preferred_element_type=f32).astype(bf16)
        for g in range(4):
            k_s[g, sl, :] = k[:, g * 128:(g + 1) * 128]

    def proj_t(i):
        sl = pl.ds(i * TQ, TQ)
        t = lax.dot_general(wt_s[...], xn_s[sl, :], (((1,), (1,)), ((), ())),
                            preferred_element_type=f32)
        qt_s[i] = (t[0:D] * (0.25 * LOG2E)).astype(bf16)
        vt_s[i] = t[D:2 * D].astype(bf16)
        r_s[:, sl] = t[2 * D:2 * D + 8]

    x_cp[0].start()
    for cp in w_cp:
        cp.start()
    wr_cp.start()
    for i in range(1, NQ):
        x_cp[i].start()
    for cp in late_cp:
        cp.start()
    x_cp[0].wait()
    layernorm(0)
    w_cp[0].wait()
    proj_k(0)
    w_cp[1].wait()
    w_cp[2].wait()
    wr_cp.wait()
    wt_s[0:D, :] = wq_s[...].T
    wt_s[D:2 * D, :] = wv_s[...].T
    wt_s[2 * D:MT, :] = jnp.broadcast_to(wr_ref[...].astype(f32).reshape(1, D), (16, D)).astype(bf16)
    for i in range(1, NQ):
        x_cp[i].wait()
        layernorm(i)
        proj_t(i - 1)
        proj_k(i)
    proj_t(NQ - 1)
    sbuf[1][U - 1][pl.ds((NC - 1) * KC, KC), :] = jnp.zeros((KC, TQ), f32)
    mpbuf[1][...] = jnp.zeros((8, TQ), f32)
    zero_s[...] = jnp.zeros((DH, TQ), f32)
    w0buf[0][...] = get_w(U)[1]
    for cp in late_cp:
        cp.wait()
    r = r_s[...].astype(bf16).astype(f32)
    r = jnp.where(r != r, -jnp.inf, r)
    rmax = jnp.max(r, axis=1, keepdims=True)
    lane = lax.broadcasted_iota(jnp.int32, (8, S), 1)
    idx = jnp.min(jnp.where(r == rmax, lane, S), axis=1, keepdims=True)
    onehot = jnp.where(lane == idx, 1.0, 0.0).astype(bf16)
    idx_s[...] = jnp.broadcast_to(idx, (8, 128))
    st = {}

    def ex_sel(c):
        part = jnp.dot(onehot[:, c * 256:(c + 1) * 256], xn_s[pl.ds(c * 256, 256), :],
                       preferred_element_type=f32)
        st['xsel'] = part if c == 0 else st['xsel'] + part

    nsplit = [0, 512, 1024, 1536, 1792]

    def ex_gu(c):
        if c == 0:
            st['xs'] = st['xsel'].astype(bf16)
        wref = wg_s if c < 4 else wu_s
        j = c % 4
        st[c] = jnp.dot(st['xs'], wref[:, nsplit[j]:nsplit[j + 1]],
                        preferred_element_type=f32).astype(bf16).astype(f32)

    def ex_down(c):
        if c == 0:
            a = jnp.concatenate([st[j] for j in range(4)], axis=1)
            u_ = jnp.concatenate([st[4 + j] for j in range(4)], axis=1)
            gte = (a * jax.nn.sigmoid(a)).astype(bf16).astype(f32)
            st['gu'] = (gte * u_).astype(bf16)
        if c < 7:
            part = jnp.dot(st['gu'][:, c * 256:(c + 1) * 256], wd_s[pl.ds(c * 256, 256), :],
                           preferred_element_type=f32)
            st['y'] = part if c == 0 else st['y'] + part

    extras = [None] * (U - 3) + [ex_sel, ex_gu, ex_down]
    for u in range(U):
        produce_only(u, sbuf[0][u], mbuf[0][u], extras[u])
    y = st['y'].astype(bf16).astype(f32)
    rs = jax.nn.sigmoid(rmax).astype(bf16).astype(f32)
    y_s[...] = (y * rs).astype(bf16).astype(f32)

    def body(gb, carry):
        carry = lax.cond(
            gb % 2 == 0,
            lambda a, l: block(gb, 0, a, l),
            lambda a, l: block(gb, 1, a, l),
            *carry)

        @pl.when(jnp.logical_and(gb % NB == 0, jnp.logical_and(gb > 0, gb < (NQ - NDEF) * NB)))
        def _():
            epilogue(gb // NB - 1)

        return carry

    init = (jnp.zeros((DH, TQ), f32), jnp.ones((8, TQ), f32))
    acc_p, lsum_p = lax.fori_loop(0, NGB - 1, body, init)

    qas = list(range(NQ - 1 - NDEF, NQ - 1))
    qb = NQ - 1

    RP = 64
    NKA = D // 128
    NKB = KPART // 128
    pieces = [(qa, j, kt) for qa in qas for j in range(TQ // RP) for kt in range(NKA)]
    pieces += [(qb, j, kt) for j in range(TQ // RP) for kt in range(NKB)]
    nslot = U * NC
    pacc = {}

    def mk_ex(u):
        def ex(c):
            s = u * NC + c
            lo = (s * len(pieces)) // nslot
            hi = ((s + 1) * len(pieces)) // nslot
            for (q, j, kt) in pieces[lo:hi]:
                r = lax.dot_general(ot_s[q, pl.ds(kt * 128, 128), pl.ds(j * RP, RP)],
                                    wo_s[pl.ds(kt * 128, 128), :], tn, preferred_element_type=f32)
                pacc[0] = r if kt == 0 else pacc[0] + r
                if q != qb and kt == NKA - 1:
                    out_rows(q, j * RP, RP, pacc[0])
                    if j == TQ // RP - 1:
                        out_cp(q).start()
                if q == qb and kt == NKB - 1:
                    part_s[pl.ds(j * RP, RP), :] = pacc[0]
        return ex

    lb = NGB - 1
    lp = lb % 2
    acc_p, lsum_p = block(lb, lp, acc_p, lsum_p, produce=False,
                          extras=[mk_ex(u) for u in range(U)])
    m_prev = mpbuf[lp][...]
    p, lsum_p = p_chunk(NC - 1, sbuf[lp][U - 1], m_prev, lsum_p)
    acc_p = pv_chunk(NQ * H - 1, NC - 1, p, acc_p)
    finalize(NQ * H - 1, acc_p, lsum_p)
    attn = part_s[...] + lax.dot_general(ot_s[qb, pl.ds(KPART, D - KPART), :],
                                         wo_s[pl.ds(KPART, D - KPART), :], tn,
                                         preferred_element_type=f32)
    out_rows(qb, 0, TQ, attn)
    out_cp(qb).start()
    for q in range(NQ):
        out_cp(q).wait()


@jax.jit
def pallas_parallel_sum__softmax_full_mha__moe_arch_mod__prompt_kernel(
    A_x, A_wqkv, A_wo, B_x, B_w_r, B_w_gate, B_w_up, B_w_down,
):
    x = A_x.reshape(S, D)
    wr = B_w_r
    anyspec = pl.BlockSpec(memory_space=pl.ANY)
    out = pl.pallas_call(
        _kernel,
        in_specs=[anyspec, anyspec, anyspec,
                  anyspec, anyspec, anyspec, anyspec],
        out_specs=anyspec,
        out_shape=jax.ShapeDtypeStruct((S, D), bf16),
        scratch_shapes=[
            pltpu.VMEM((S, D), bf16),
            pltpu.VMEM((D, D), bf16),
            pltpu.VMEM((D, D), bf16),
            pltpu.VMEM((D, D), bf16),
            pltpu.VMEM((MT, D), bf16),
            pltpu.VMEM((S, D), bf16),
            pltpu.VMEM((4, S, 128), bf16),
            pltpu.VMEM((NQ, D, TQ), bf16),
            pltpu.VMEM((NQ, D, TQ), bf16),
            pltpu.VMEM((8, S), f32),
            pltpu.VMEM((NQ, D, TQ), bf16),
            pltpu.VMEM((8, D), f32),
            pltpu.VMEM((8, 128), jnp.int32),
            pltpu.VMEM((D, D), bf16),
            pltpu.VMEM((D, F), bf16),
            pltpu.VMEM((D, F), bf16),
            pltpu.VMEM((F, D), bf16),
            pltpu.VMEM((S, D), bf16),
            pltpu.VMEM((TQ, D), f32),
            pltpu.VMEM((D,), bf16),
            pltpu.VMEM((128, TQ), bf16),
            pltpu.VMEM((128, TQ), bf16),
            pltpu.VMEM((8, TQ), f32),
            pltpu.VMEM((8, TQ), f32),
            pltpu.VMEM((DH, TQ), f32),
            pltpu.SemaphoreType.DMA((NQ + 8,)),
            pltpu.SemaphoreType.DMA((NQ,)),
        ] + [pltpu.VMEM((S, TQ), f32) for _ in range(2 * U)]
          + [pltpu.VMEM((8, TQ), f32) for _ in range(2 * U)],
        compiler_params=pltpu.CompilerParams(
            vmem_limit_bytes=110 * 1024 * 1024,
        ),
    )(x, A_wqkv, wr, A_wo, B_w_gate, B_w_up, B_w_down)
    return out.reshape(1, S, D)
```
